```python
import os as _os
_os.environ.setdefault("JAX_PLATFORMS", "cpu")
import jax
import jax.numpy as jnp

def _softmax(x, axis=-1):
    return jax.nn.softmax(x, axis=axis)
def _gelu(x):
    return jax.nn.gelu(x, approximate=True)
def _silu(x):
    return jax.nn.silu(x)
def _sigmoid(x):
    return jax.nn.sigmoid(x)
def _layernorm(x, axis=-1, eps=1e-5):
    m = jnp.mean(x, axis=axis, keepdims=True)
    v = jnp.var(x, axis=axis, keepdims=True)
    return (x - m) / jnp.sqrt(v + eps)
def _scatter_add(tgt, idx, src, axis=0):
    return tgt.at[idx].add(src)
def _segment_sum(src, seg, n):
    return jax.ops.segment_sum(src, seg, n)
class _Rng:
    def __init__(self, key):
        self._k = key
    def _next(self):
        self._k, sub = jax.random.split(self._k)
        return sub
    def normal(self, shape):
        return jax.random.normal(self._next(), shape, dtype=jnp.bfloat16)
    def randint(self, lo, hi, shape):
        return jax.random.randint(self._next(), shape, lo, hi, dtype=jnp.int32)
    def uniform(self, shape, lo=0.0, hi=1.0):
        return jax.random.uniform(self._next(), shape, jnp.bfloat16, lo, hi)
    def permutation(self, n):
        return jax.random.permutation(self._next(), n)


kernel_name = 'standalone__mha_softmax__near_ridge'

def setup_inputs():
    _rng = _Rng(jax.random.key(int.from_bytes(__import__("os").urandom(4), "little")))
    _w = (lambda a: (lambda t: t.astype(jnp.bfloat16) if jnp.issubdtype(t.dtype, jnp.floating) else t)(jnp.asarray(a)))
    B, H, Sq, Sk, D = 16, 16, 256, 256, 256
    return {
        "q": _w((lambda *s: _rng.normal(s) * 0.4)(B, H, Sq, D)),
        "k": _w((lambda *s: _rng.normal(s) * 0.4)(B, H, Sk, D)),
        "v": _w((lambda *s: _rng.normal(s) * 0.05)(B, H, Sk, D)),
    }

def reference(q, k, v):
    scale = q.shape[-1] ** -0.5
    scores = jnp.einsum("bhqd,bhkd->bhqk", q, k) * scale
    p = _softmax(scores, axis=-1)
    return jnp.einsum("bhqk,bhkd->bhqd", p, v)
```

```python
import math

import jax
import jax.numpy as jnp
import jax.experimental.pallas as pl
import jax.experimental.pallas.tpu as pltpu

_LOG2E = math.log2(math.e)

_G = 4
_R = 3
_X = 32
_NY = 64


def _attention_head(q, k, v, scale):
    s = jax.lax.dot_general(
        q, k, (((1,), (1,)), ((), ())), preferred_element_type=jnp.float32)
    m = jnp.max(s, axis=-1, keepdims=True)
    p = jnp.exp2((s - m) * (scale * _LOG2E))
    l = jnp.sum(p, axis=-1, keepdims=True)
    o = jnp.dot(p.astype(v.dtype), v, preferred_element_type=jnp.float32)
    return (o * (1.0 / l)).astype(q.dtype)


@jax.jit
def pallas_standalone__mha_softmax__near_ridge_kernel(
    q: jax.Array,
    k: jax.Array,
    v: jax.Array,
):
    B, H, Sq, D = q.shape
    Sk = k.shape[2]
    N = B * H
    G, R, X, ny = _G, _R, _X, _NY
    assert N % X == 0 and X % G == 0 and Sq % ny == 0
    HPG = N // X
    XB = X // G
    NS = N // G
    nw = Sq // ny
    lag = R - 1
    scale = D ** -0.5

    def kernel(q_hbm, k_hbm, v_hbm, o_hbm, qb, kb, vb, ob, rsem, wsem):
        def reads(i, slot):
            hh, xb = i // XB, i % XB
            return [
                pltpu.make_async_copy(
                    src.at[pl.ds(xb * G, G), hh], buf.at[slot], rsem.at[a, slot])
                for a, (src, buf) in enumerate(
                    ((q_hbm, qb), (k_hbm, kb), (v_hbm, vb)))
            ]

        def write(hh, j):
            rows = pl.ds(j * ny, ny)
            return pltpu.make_async_copy(
                ob.at[:, hh, rows], o_hbm.at[:, hh, rows], wsem.at[hh])

        for j in range(lag):
            for c in reads(j, j % R):
                c.start()

        def body(i, carry):
            slot = i % R

            @pl.when(i + lag < NS)
            def _():
                for c in reads(i + lag, (i + lag) % R):
                    c.start()

            for c in reads(i, slot):
                c.wait()

            @pl.when(i == NS - 1)
            def _():
                for hh in range(HPG - 1):
                    for j in range(nw):
                        write(hh, j).start()

            hh, xb = i // XB, i % XB
            for g in range(G):
                ob[xb * G + g, hh] = _attention_head(
                    qb[slot, g], kb[slot, g], vb[slot, g], scale)
            return carry

        jax.lax.fori_loop(0, NS, body, ())

        for j in range(nw):
            write(HPG - 1, j).start()
        for hh in range(HPG):
            for j in range(nw):
                write(hh, j).wait()

    any_spec = pl.BlockSpec(memory_space=pl.ANY)
    out = pl.pallas_call(
        kernel,
        in_specs=[any_spec, any_spec, any_spec],
        out_specs=any_spec,
        out_shape=jax.ShapeDtypeStruct((X, HPG, Sq, D), q.dtype),
        scratch_shapes=[
            pltpu.VMEM((R, G, Sq, D), q.dtype),
            pltpu.VMEM((R, G, Sk, D), k.dtype),
            pltpu.VMEM((R, G, Sk, D), v.dtype),
            pltpu.VMEM((X, HPG, Sq, D), q.dtype),
            pltpu.SemaphoreType.DMA((3, R)),
            pltpu.SemaphoreType.DMA((HPG,)),
        ],
        compiler_params=pltpu.CompilerParams(vmem_limit_bytes=100 * 1024 * 1024),
    )(
        q.reshape(X, HPG, Sq, D),
        k.reshape(X, HPG, Sk, D),
        v.reshape(X, HPG, Sk, D),
    )
    return out.reshape(B, H, Sq, D)
```

```python
import math

import jax
import jax.numpy as jnp
import jax.experimental.pallas as pl
import jax.experimental.pallas.tpu as pltpu

_LOG2E = math.log2(math.e)

_G = 4
_R = 3
_X = 32
_NY = 64
_EARLY = 2


def _attention_head(q, k, v, scale):
    s = jax.lax.dot_general(
        q, k, (((1,), (1,)), ((), ())), preferred_element_type=jnp.float32)
    m = jnp.max(s, axis=-1, keepdims=True)
    p = jnp.exp2((s - m) * (scale * _LOG2E))
    l = jnp.sum(p, axis=-1, keepdims=True)
    o = jnp.dot(p.astype(v.dtype), v, preferred_element_type=jnp.float32)
    return (o * (1.0 / l)).astype(q.dtype)


@jax.jit
def pallas_standalone__mha_softmax__near_ridge_kernel(
    q: jax.Array,
    k: jax.Array,
    v: jax.Array,
):
    B, H, Sq, D = q.shape
    Sk = k.shape[2]
    N = B * H
    G, R, X, ny = _G, _R, _X, _NY
    assert N % X == 0 and X % G == 0 and Sq % ny == 0
    HPG = N // X
    XB = X // G
    NS = N // G
    nw = Sq // ny
    lag = R - 1
    scale = D ** -0.5
    assert HPG >= 2 and NS > lag
    ready = [(hh, j) for hh in range(HPG - 1) for j in range(nw)]

    def kernel(q_hbm, k_hbm, v_hbm, o_hbm, qb, kb, vb, ob, rsem, wsem):
        def reads(i, slot):
            hh, xb = i // XB, i % XB
            return [
                pltpu.make_async_copy(
                    src.at[pl.ds(xb * G, G), hh], buf.at[slot], rsem.at[a, slot])
                for a, (src, buf) in enumerate(
                    ((q_hbm, qb), (k_hbm, kb), (v_hbm, vb)))
            ]

        def write(hh, j):
            rows = pl.ds(j * ny, ny)
            return pltpu.make_async_copy(
                ob.at[:, hh, rows], o_hbm.at[:, hh, rows], wsem)

        for j in range(lag):
            for c in reads(j, j % R):
                c.start()

        def body(i, carry):
            slot = i % R

            @pl.when(i + lag < NS)
            def _():
                for c in reads(i + lag, (i + lag) % R):
                    c.start()

            @pl.when(i == NS - 1)
            def _():
                for hh, j in ready[:_EARLY]:
                    write(hh, j).start()

            for c in reads(i, slot):
                c.wait()

            @pl.when(i == NS - 1)
            def _():
                for hh, j in ready[_EARLY:]:
                    write(hh, j).start()

            hh, xb = i // XB, i % XB
            for g in range(G):
                ob[xb * G + g, hh] = _attention_head(
                    qb[slot, g], kb[slot, g], vb[slot, g], scale)
            return carry

        jax.lax.fori_loop(0, NS, body, ())

        for j in range(nw):
            write(HPG - 1, j).start()
        pltpu.make_async_copy(ob, o_hbm, wsem).wait()

    any_spec = pl.BlockSpec(memory_space=pl.ANY)
    out = pl.pallas_call(
        kernel,
        in_specs=[any_spec, any_spec, any_spec],
        out_specs=any_spec,
        out_shape=jax.ShapeDtypeStruct((X, HPG, Sq, D), q.dtype),
        scratch_shapes=[
            pltpu.VMEM((R, G, Sq, D), q.dtype),
            pltpu.VMEM((R, G, Sk, D), k.dtype),
            pltpu.VMEM((R, G, Sk, D), v.dtype),
            pltpu.VMEM((X, HPG, Sq, D), q.dtype),
            pltpu.SemaphoreType.DMA((3, R)),
            pltpu.SemaphoreType.DMA(()),
        ],
        compiler_params=pltpu.CompilerParams(vmem_limit_bytes=64 * 1024 * 1024),
    )(
        q.reshape(X, HPG, Sq, D),
        k.reshape(X, HPG, Sk, D),
        v.reshape(X, HPG, Sk, D),
    )
    return out.reshape(B, H, Sq, D)
```

```python
import math

import jax
import jax.numpy as jnp
import jax.experimental.pallas as pl
import jax.experimental.pallas.tpu as pltpu

_LOG2E = math.log2(math.e)

_G = 4
_R = 3
_X = 16
_NY = 32


def _attention_head(q, k, v, scale):
    s = jax.lax.dot_general(
        q, k, (((1,), (1,)), ((), ())), preferred_element_type=jnp.float32)
    m = jnp.max(s, axis=-1, keepdims=True)
    p = jnp.exp2((s - m) * (scale * _LOG2E))
    l = jnp.sum(p, axis=-1, keepdims=True)
    o = jnp.dot(p.astype(v.dtype), v, preferred_element_type=jnp.float32)
    return (o * (1.0 / l)).astype(q.dtype)


@jax.jit
def pallas_standalone__mha_softmax__near_ridge_kernel(
    q: jax.Array,
    k: jax.Array,
    v: jax.Array,
):
    B, H, Sq, D = q.shape
    Sk = k.shape[2]
    N = B * H
    G, R, X, ny = _G, _R, _X, _NY
    assert N % X == 0 and X % G == 0 and Sq % ny == 0
    HPG = N // X
    XB = X // G
    NS = N // G
    nw = Sq // ny
    lag = R - 1
    scale = D ** -0.5
    assert NS > lag

    def kernel(q_hbm, k_hbm, v_hbm, o_hbm, qb, kb, vb, ob, rsem, wsem):
        def reads(i, slot):
            hh, xb = i // XB, i % XB
            return [
                pltpu.make_async_copy(
                    src.at[pl.ds(xb * G, G), hh], buf.at[slot], rsem.at[a, slot])
                for a, (src, buf) in enumerate(
                    ((q_hbm, qb), (k_hbm, kb), (v_hbm, vb)))
            ]

        def start_writes(lo, hi):
            def start(t, carry):
                hh = t // nw
                rows = pl.ds(pl.multiple_of((t % nw) * ny, ny), ny)
                pltpu.make_async_copy(
                    ob.at[:, hh, rows], o_hbm.at[:, hh, rows], wsem).start()
                return carry
            jax.lax.fori_loop(lo, hi, start, ())

        for j in range(lag):
            for c in reads(j, j % R):
                c.start()

        def body(i, carry):
            slot = i % R

            @pl.when(i + lag < NS)
            def _():
                for c in reads(i + lag, (i + lag) % R):
                    c.start()

            @pl.when(i == NS - 1)
            def _():
                start_writes(0, (HPG - 1) * nw)

            for c in reads(i, slot):
                c.wait()

            hh, xb = i // XB, i % XB
            for g in range(G):
                ob[xb * G + g, hh] = _attention_head(
                    qb[slot, g], kb[slot, g], vb[slot, g], scale)
            return carry

        jax.lax.fori_loop(0, NS, body, ())

        start_writes((HPG - 1) * nw, HPG * nw)
        pltpu.make_async_copy(ob, o_hbm, wsem).wait()

    any_spec = pl.BlockSpec(memory_space=pl.ANY)
    out = pl.pallas_call(
        kernel,
        in_specs=[any_spec, any_spec, any_spec],
        out_specs=any_spec,
        out_shape=jax.ShapeDtypeStruct((X, HPG, Sq, D), q.dtype),
        scratch_shapes=[
            pltpu.VMEM((R, G, Sq, D), q.dtype),
            pltpu.VMEM((R, G, Sk, D), k.dtype),
            pltpu.VMEM((R, G, Sk, D), v.dtype),
            pltpu.VMEM((X, HPG, Sq, D), q.dtype),
            pltpu.SemaphoreType.DMA((3, R)),
            pltpu.SemaphoreType.DMA(()),
        ],
        compiler_params=pltpu.CompilerParams(vmem_limit_bytes=64 * 1024 * 1024),
    )(
        q.reshape(X, HPG, Sq, D),
        k.reshape(X, HPG, Sk, D),
        v.reshape(X, HPG, Sk, D),
    )
    return out.reshape(B, H, Sq, D)
```

```python
import math

import jax
import jax.numpy as jnp
import jax.experimental.pallas as pl
import jax.experimental.pallas.tpu as pltpu

_LOG2E = math.log2(math.e)

_G = 8
_R = 3
_NY = 16


def _attention_head(q, k, v, scale):
    s = jax.lax.dot_general(
        q, k, (((1,), (1,)), ((), ())), preferred_element_type=jnp.float32)
    m = jnp.max(s, axis=-1, keepdims=True)
    p = jnp.exp2((s - m) * (scale * _LOG2E))
    l = jnp.sum(p, axis=-1, keepdims=True)
    o = jnp.dot(p.astype(v.dtype), v, preferred_element_type=jnp.float32)
    return (o * (1.0 / l)).astype(q.dtype)


@jax.jit
def pallas_standalone__mha_softmax__near_ridge_kernel(
    q: jax.Array,
    k: jax.Array,
    v: jax.Array,
):
    B, H, Sq, D = q.shape
    Sk = k.shape[2]
    G, R, ny = _G, _R, _NY
    NC = (B * H) // G
    nw = Sq // ny
    lag = R - 1
    scale = D ** -0.5
    assert (B * H) % G == 0 and Sq % ny == 0 and NC > lag

    def kernel(q_hbm, k_hbm, v_hbm, o_hbm, qb, kb, vb, ob, rsem, wsem):
        def reads(c, slot):
            return [
                pltpu.make_async_copy(src.at[:, c], buf.at[slot], rsem.at[slot])
                for src, buf in ((q_hbm, qb), (k_hbm, kb), (v_hbm, vb))
            ]

        def start_writes(lo, hi):
            def start(t, carry):
                c = t // nw
                rows = pl.ds(pl.multiple_of((t % nw) * ny, ny), ny)
                pltpu.make_async_copy(
                    ob.at[:, c, rows], o_hbm.at[:, c, rows], wsem).start()
                return carry
            jax.lax.fori_loop(lo, hi, start, ())

        for c in range(lag):
            for copy in reads(c, c % R):
                copy.start()

        def body(c, carry):
            slot = c % R

            @pl.when(c + lag < NC)
            def _():
                for copy in reads(c + lag, (c + lag) % R):
                    copy.start()

            @pl.when(c == NC - 1)
            def _():
                start_writes(0, (NC - 1) * nw)

            for copy in reads(c, slot):
                copy.wait()

            for x in range(G):
                ob[x, c] = _attention_head(
                    qb[slot, x], kb[slot, x], vb[slot, x], scale)
            return carry

        jax.lax.fori_loop(0, NC, body, ())

        start_writes((NC - 1) * nw, NC * nw)
        pltpu.make_async_copy(ob, o_hbm, wsem).wait()

    any_spec = pl.BlockSpec(memory_space=pl.ANY)
    out = pl.pallas_call(
        kernel,
        in_specs=[any_spec, any_spec, any_spec],
        out_specs=any_spec,
        out_shape=jax.ShapeDtypeStruct((G, NC, Sq, D), q.dtype),
        scratch_shapes=[
            pltpu.VMEM((R, G, Sq, D), q.dtype),
            pltpu.VMEM((R, G, Sk, D), k.dtype),
            pltpu.VMEM((R, G, Sk, D), v.dtype),
            pltpu.VMEM((G, NC, Sq, D), q.dtype),
            pltpu.SemaphoreType.DMA((R,)),
            pltpu.SemaphoreType.DMA(()),
        ],
        compiler_params=pltpu.CompilerParams(vmem_limit_bytes=64 * 1024 * 1024),
    )(
        q.reshape(G, NC, Sq, D),
        k.reshape(G, NC, Sk, D),
        v.reshape(G, NC, Sk, D),
    )
    return out.reshape(B, H, Sq, D)
```
